```python
import os as _os
_os.environ.setdefault("JAX_PLATFORMS", "cpu")
import jax
import jax.numpy as jnp

def _softmax(x, axis=-1):
    return jax.nn.softmax(x, axis=axis)
def _gelu(x):
    return jax.nn.gelu(x, approximate=True)
def _silu(x):
    return jax.nn.silu(x)
def _sigmoid(x):
    return jax.nn.sigmoid(x)
def _layernorm(x, axis=-1, eps=1e-5):
    m = jnp.mean(x, axis=axis, keepdims=True)
    v = jnp.var(x, axis=axis, keepdims=True)
    return (x - m) / jnp.sqrt(v + eps)
def _scatter_add(tgt, idx, src, axis=0):
    return tgt.at[idx].add(src)
def _segment_sum(src, seg, n):
    return jax.ops.segment_sum(src, seg, n)
class _Rng:
    def __init__(self, key):
        self._k = key
    def _next(self):
        self._k, sub = jax.random.split(self._k)
        return sub
    def normal(self, shape):
        return jax.random.normal(self._next(), shape, dtype=jnp.bfloat16)
    def randint(self, lo, hi, shape):
        return jax.random.randint(self._next(), shape, lo, hi, dtype=jnp.int32)
    def uniform(self, shape, lo=0.0, hi=1.0):
        return jax.random.uniform(self._next(), shape, jnp.bfloat16, lo, hi)
    def permutation(self, n):
        return jax.random.permutation(self._next(), n)


kernel_name = 'standalone__sliding_local_fixed_window__prompt'

def setup_inputs():
    _rng = _Rng(jax.random.key(int.from_bytes(__import__("os").urandom(4), "little")))
    _w = (lambda a: (lambda t: t.astype(jnp.bfloat16) if jnp.issubdtype(t.dtype, jnp.floating) else t)(jnp.asarray(a)))
    B, H, S, D = 1, 32, 2048, 128
    return {
        "q": _w((lambda *s: _rng.normal(s) * 0.4)(B, H, S, D)),
        "k": _w((lambda *s: _rng.normal(s) * 0.4)(B, H, S, D)),
        "v": _w((lambda *s: _rng.normal(s) * 0.05)(B, H, S, D)),
    }

def reference(q, k, v):
    B, H, S, D = q.shape
    w = 32
    pos = jnp.arange(S)
    rel = pos[:, None] - pos[None, :]
    mask = (rel >= 0) & (rel < w)
    scores = jnp.einsum("bhqd,bhkd->bhqk", q, k) * (D ** -0.5)
    scores = jnp.where(mask[None, None], scores, (lambda x, dt: x.astype(dt))(jnp.array(-1e9), q.dtype))
    p = _softmax(scores, axis=-1)
    return jnp.einsum("bhqk,bhkd->bhqd", p, v)
```

```python
import math

import jax
import jax.numpy as jnp
from jax import lax
import jax.experimental.pallas as pl
import jax.experimental.pallas.tpu as pltpu

_W = 32
_T = 128
_MASKED = -998244352.0
_NEG = -1e30
_NT = (((1,), (1,)), ((), ()))


def _banded_head(q_ref, k_ref, v_ref, o_ref):
    seq, dim = q_ref.shape
    c = float(dim**-0.5 * math.log2(math.e))
    half = _T // 2
    row = lax.broadcasted_iota(jnp.int32, (half, _T), 0)
    lane = lax.broadcasted_iota(jnp.int32, (half, _T), 1)
    d = lane - row

    def probs(i):
        qi = q_ref[pl.ds(_T * i, _T), :]
        lo = _W if i else 0
        kk = k_ref[pl.ds(_T * i - lo, _T + lo), :]
        st = lax.dot_general(kk, qi, _NT, preferred_element_type=jnp.float32)
        s = jnp.where(d < 48, st[lo : lo + half], st[lo + half :])
        if i:
            top = jnp.where(d[_W:] < -16, st[:_W], s[_W:])
            s = jnp.concatenate([s[:_W], top], axis=0)
            s = jnp.where((d & (half - 1)) < _W, s, _NEG)
        else:
            s = jnp.where(((d & (half - 1)) < _W) & (d >= 0), s, _NEG)
        m = jnp.max(s, axis=0, keepdims=True)
        e = jnp.exp2((s - m) * c)
        p = e * (1.0 / jnp.sum(e, axis=0, keepdims=True))
        first = (d >= 0) & (d < 48)
        pt = jnp.concatenate(
            [jnp.where(first, p, 0.0), jnp.where(first, 0.0, p)], axis=0
        )
        return pt.astype(jnp.bfloat16).T, m

    n = seq // _T
    cur, low = probs(0)
    carry = None
    for i in range(1, n + 1):
        lhs = cur
        if i < n:
            p, m = probs(i)
            low = jnp.minimum(low, m)
            head = p[:_W].astype(jnp.float32)
            back = d[:_W] > 0
            prev = jnp.where(back, head, 0.0).astype(jnp.bfloat16)
            here = jnp.where(back, 0.0, head).astype(jnp.bfloat16)
            lhs = jnp.concatenate([cur, prev], axis=0)
            cur = jnp.concatenate([here, p[_W:]], axis=0)
        o = jnp.dot(
            lhs,
            v_ref[pl.ds(_T * (i - 1), _T), :],
            preferred_element_type=jnp.float32,
        )
        out = o[:_T]
        if carry is not None:
            out = jnp.concatenate([o[:_W] + carry, o[_W:_T]], axis=0)
        o_ref[pl.ds(_T * (i - 1), _T), :] = out.astype(o_ref.dtype)
        if i < n:
            carry = o[_T:]
    return low


def _dense_head(q_ref, k_ref, v_ref, o_ref):
    seq, dim = q_ref.shape
    rows = 16

    def body(i, _):
        r0 = pl.multiple_of(i * rows, rows)
        s = lax.dot_general(
            q_ref[pl.ds(r0, rows), :], k_ref[...], _NT,
            preferred_element_type=jnp.float32,
        )
        s = s.astype(jnp.bfloat16).astype(jnp.float32) * float(dim**-0.5)
        s = s.astype(jnp.bfloat16).astype(jnp.float32)
        rel = (
            r0
            + lax.broadcasted_iota(jnp.int32, s.shape, 0)
            - lax.broadcasted_iota(jnp.int32, s.shape, 1)
        )
        s = jnp.where((rel >= 0) & (rel < _W), s, _MASKED)
        e = jnp.exp(s - jnp.max(s, axis=1, keepdims=True))
        p = e / jnp.sum(e, axis=1, keepdims=True)
        o = jnp.dot(
            p.astype(jnp.bfloat16), v_ref[...], preferred_element_type=jnp.float32
        )
        o_ref[pl.ds(r0, rows), :] = o.astype(o_ref.dtype)

    lax.fori_loop(0, seq // rows, body, None)


@jax.jit
def pallas_standalone__sliding_local_fixed_window__prompt_kernel(
    q: jax.Array,
    k: jax.Array,
    v: jax.Array,
):
    batch, heads, seq, dim = q.shape
    assert batch == 1 and dim == _T and seq % _T == 0 and heads % 4 == 0
    chunks = 4
    hpc = heads // chunks
    early = heads - hpc
    tail = 128
    run = 32

    def kernel(q_hbm, k_hbm, v_hbm, o_hbm, qb, kb, vb, ob, rsem, wsem):
        def reads(c):
            hs = pl.ds(c * hpc, hpc)
            rows = pl.ds(0, seq - tail if c == chunks - 1 else seq)
            return [
                pltpu.make_async_copy(q_hbm.at[0, hs], qb.at[hs], rsem.at[c]),
                pltpu.make_async_copy(k_hbm.at[0, hs], kb.at[hs], rsem.at[c]),
                pltpu.make_async_copy(
                    v_hbm.at[0, hs, rows], vb.at[hs, rows], rsem.at[c]
                ),
            ]

        def tail_read():
            hs, rows = pl.ds(early, hpc), pl.ds(seq - tail, tail)
            return pltpu.make_async_copy(
                v_hbm.at[0, hs, rows], vb.at[hs, rows], rsem.at[chunks]
            )

        def start_writes(h0, n):
            def one(j, _):
                hs, rows = pl.ds(h0, n), pl.ds(pl.multiple_of(j * run, run), run)
                pltpu.make_async_copy(
                    ob.at[hs, rows], o_hbm.at[0, hs, rows], wsem
                ).start()

            lax.fori_loop(0, seq // run, one, None, unroll=8)

        for c in range(chunks):
            for copy in reads(c):
                copy.start()
        tail_read().start()

        def head(h, _):
            for c in range(chunks):

                @pl.when(h == c * hpc)
                def _():
                    for copy in reads(c):
                        copy.wait()
                    if c == chunks - 1:
                        start_writes(0, early)
                        tail_read().wait()

            refs = (qb.at[h], kb.at[h], vb.at[h], ob.at[h])
            low = _banded_head(*refs)

            @pl.when(jnp.min(low) * float(dim**-0.5) < 0.5 * _MASKED)
            def _():
                _dense_head(*refs)

        lax.fori_loop(0, heads, head, None)
        start_writes(early, hpc)
        pltpu.make_async_copy(ob, o_hbm.at[0], wsem).wait()

    buf = pltpu.VMEM((heads, seq, dim), q.dtype)
    return pl.pallas_call(
        kernel,
        in_specs=[pl.BlockSpec(memory_space=pl.ANY)] * 3,
        out_specs=pl.BlockSpec(memory_space=pl.ANY),
        out_shape=jax.ShapeDtypeStruct(q.shape, q.dtype),
        scratch_shapes=[
            buf,
            buf,
            buf,
            buf,
            pltpu.SemaphoreType.DMA((chunks + 1,)),
            pltpu.SemaphoreType.DMA,
        ],
        compiler_params=pltpu.CompilerParams(vmem_limit_bytes=100 * 2**20),
    )(q, k, v)
```

```python
import math

import numpy as np
import jax
import jax.numpy as jnp
from jax import lax
import jax.experimental.pallas as pl
import jax.experimental.pallas.tpu as pltpu

_W = 32
_T = 128
_MASKED = -998244352.0
_NEG = -1e30
_NT = (((1,), (1,)), ((), ()))


def _banded_head(q_ref, k_ref, v_ref, o_ref):
    seq, dim = q_ref.shape
    c = float(dim**-0.5 * math.log2(math.e))
    half = _T // 2
    row = lax.broadcasted_iota(jnp.int32, (half, _T), 0)
    lane = lax.broadcasted_iota(jnp.int32, (half, _T), 1)
    d = lane - row

    def probs(i):
        qi = q_ref[pl.ds(_T * i, _T), :]
        lo = _W if i else 0
        kk = k_ref[pl.ds(_T * i - lo, _T + lo), :]
        st = lax.dot_general(kk, qi, _NT, preferred_element_type=jnp.float32)
        s = jnp.where(d < 48, st[lo : lo + half], st[lo + half :])
        if i:
            top = jnp.where(d[_W:] < -16, st[:_W], s[_W:])
            s = jnp.concatenate([s[:_W], top], axis=0)
            s = jnp.where((d & (half - 1)) < _W, s, _NEG)
        else:
            s = jnp.where(((d & (half - 1)) < _W) & (d >= 0), s, _NEG)
        m = jnp.max(s, axis=0, keepdims=True)
        e = jnp.exp2((s - m) * c)
        p = e * (1.0 / jnp.sum(e, axis=0, keepdims=True))
        first = (d >= 0) & (d < 48)
        pt = jnp.concatenate(
            [jnp.where(first, p, 0.0), jnp.where(first, 0.0, p)], axis=0
        )
        return pt.astype(jnp.bfloat16).T, m

    n = seq // _T
    cur, low = probs(0)
    carry = None
    for i in range(1, n + 1):
        lhs = cur
        if i < n:
            p, m = probs(i)
            low = jnp.minimum(low, m)
            head = p[:_W].astype(jnp.float32)
            back = d[:_W] > 0
            prev = jnp.where(back, head, 0.0).astype(jnp.bfloat16)
            here = jnp.where(back, 0.0, head).astype(jnp.bfloat16)
            lhs = jnp.concatenate([cur, prev], axis=0)
            cur = jnp.concatenate([here, p[_W:]], axis=0)
        o = jnp.dot(
            lhs,
            v_ref[pl.ds(_T * (i - 1), _T), :],
            preferred_element_type=jnp.float32,
        )
        out = o[:_T]
        if carry is not None:
            out = jnp.concatenate([o[:_W] + carry, o[_W:_T]], axis=0)
        o_ref[pl.ds(_T * (i - 1), _T), :] = out.astype(o_ref.dtype)
        if i < n:
            carry = o[_T:]
    return low


def _dense_head(q_ref, k_ref, v_ref, o_ref):
    seq, dim = q_ref.shape
    rows = 16

    def body(i, _):
        r0 = pl.multiple_of(i * rows, rows)
        s = lax.dot_general(
            q_ref[pl.ds(r0, rows), :], k_ref[...], _NT,
            preferred_element_type=jnp.float32,
        )
        s = s.astype(jnp.bfloat16).astype(jnp.float32) * float(
            np.asarray(dim**-0.5, dtype=jnp.bfloat16)
        )
        s = s.astype(jnp.bfloat16).astype(jnp.float32)
        rel = (
            r0
            + lax.broadcasted_iota(jnp.int32, s.shape, 0)
            - lax.broadcasted_iota(jnp.int32, s.shape, 1)
        )
        s = jnp.where((rel >= 0) & (rel < _W), s, _MASKED)
        e = jnp.exp(s - jnp.max(s, axis=1, keepdims=True))
        p = e / jnp.sum(e, axis=1, keepdims=True)
        o = jnp.dot(
            p.astype(jnp.bfloat16), v_ref[...], preferred_element_type=jnp.float32
        )
        o_ref[pl.ds(r0, rows), :] = o.astype(o_ref.dtype)

    lax.fori_loop(0, seq // rows, body, None)


@jax.jit
def pallas_standalone__sliding_local_fixed_window__prompt_kernel(
    q: jax.Array,
    k: jax.Array,
    v: jax.Array,
):
    batch, heads, seq, dim = q.shape
    assert batch == 1 and dim == _T and seq % _T == 0 and heads % 4 == 0
    chunks = 4
    hpc = heads // chunks
    early = heads - hpc
    tail = 160
    run = 32

    def kernel(q_hbm, k_hbm, v_hbm, o_hbm, qb, kb, vb, ob, sems):
        def reads(c):
            sem = sems.at[c % 2]
            if c == chunks:
                hs, rows = pl.ds(early, hpc), pl.ds(seq - tail, tail)
                return [
                    pltpu.make_async_copy(v_hbm.at[0, hs, rows], vb.at[hs, rows], sem)
                ]
            hs = pl.ds(c * hpc, hpc)
            rows = pl.ds(0, seq - tail if c == chunks - 1 else seq)
            return [
                pltpu.make_async_copy(q_hbm.at[0, hs], qb.at[hs], sem),
                pltpu.make_async_copy(k_hbm.at[0, hs], kb.at[hs], sem),
                pltpu.make_async_copy(v_hbm.at[0, hs, rows], vb.at[hs, rows], sem),
            ]

        wsem = sems.at[(chunks - 1) % 2]

        def start_writes(h0, n):
            def one(j, _):
                hs, rows = pl.ds(h0, n), pl.ds(pl.multiple_of(j * run, run), run)
                pltpu.make_async_copy(
                    ob.at[hs, rows], o_hbm.at[0, hs, rows], wsem
                ).start()

            lax.fori_loop(0, seq // run, one, None, unroll=8)

        for copy in reads(0) + reads(1):
            copy.start()

        def head(h, _):
            for c in range(chunks):

                @pl.when(h == c * hpc)
                def _():
                    for copy in reads(c):
                        copy.wait()
                    if c < chunks - 1:
                        for copy in reads(c + 2):
                            copy.start()
                    else:
                        start_writes(0, early)
                        for copy in reads(chunks):
                            copy.wait()

            refs = (qb.at[h], kb.at[h], vb.at[h], ob.at[h])
            low = _banded_head(*refs)

            @pl.when(jnp.min(low) * float(dim**-0.5) < 0.5 * _MASKED)
            def _():
                _dense_head(*refs)

        lax.fori_loop(0, heads, head, None)
        start_writes(early, hpc)
        pltpu.make_async_copy(ob, o_hbm.at[0], wsem).wait()

    buf = pltpu.VMEM((heads, seq, dim), q.dtype)
    return pl.pallas_call(
        kernel,
        in_specs=[pl.BlockSpec(memory_space=pl.ANY)] * 3,
        out_specs=pl.BlockSpec(memory_space=pl.ANY),
        out_shape=jax.ShapeDtypeStruct(q.shape, q.dtype),
        scratch_shapes=[buf, buf, buf, buf, pltpu.SemaphoreType.DMA((2,))],
        compiler_params=pltpu.CompilerParams(vmem_limit_bytes=100 * 2**20),
    )(q, k, v)
```
